```python
import jax
import jax.numpy as jnp

def _softmax(x, axis=-1):
    return jax.nn.softmax(x, axis=axis)
def _gelu(x):
    return jax.nn.gelu(x, approximate=True)
def _silu(x):
    return jax.nn.silu(x)
def _sigmoid(x):
    return jax.nn.sigmoid(x)
def _layernorm(x, axis=-1, eps=1e-5):
    m = jnp.mean(x, axis=axis, keepdims=True)
    v = jnp.var(x, axis=axis, keepdims=True)
    return (x - m) / jnp.sqrt(v + eps)
def _scatter_add(tgt, idx, src, axis=0):
    return tgt.at[idx].add(src)
def _segment_sum(src, seg, n):
    return jax.ops.segment_sum(src, seg, n)
class _Rng:
    def __init__(self, key):
        self._k = key
    def _next(self):
        self._k, sub = jax.random.split(self._k)
        return sub
    def normal(self, shape):
        return jax.random.normal(self._next(), shape, dtype=jnp.bfloat16)
    def randint(self, lo, hi, shape):
        return jax.random.randint(self._next(), shape, lo, hi, dtype=jnp.int32)
    def uniform(self, shape, lo=0.0, hi=1.0):
        return jax.random.uniform(self._next(), shape, jnp.bfloat16, lo, hi)
    def permutation(self, n):
        return jax.random.permutation(self._next(), n)


kernel_name = 'sequential_preLN__grouped_kv_mqa__glu_gated_swiglu__prompt'

def _fwd_setup_inputs():
    _rng = _Rng(jax.random.key(int.from_bytes(__import__("os").urandom(4), "little")))
    _w = (lambda a: (lambda t: t.astype(jnp.bfloat16) if jnp.issubdtype(t.dtype, jnp.floating) else t)(jnp.asarray(a)))
    def _A_setup():
        B, S, D, H = 1, 2048, 512, 32
        Dh = D // H
        return {
            "x": _w((lambda *s: _rng.normal(s) * 0.05)(B, S, D)),
            "wq": _w((lambda *s: _rng.normal(s) * 0.05)(D, H * Dh)),
            "wk": _w((lambda *s: _rng.normal(s) * 0.05)(D, Dh)),
            "wv": _w((lambda *s: _rng.normal(s) * 0.05)(D, Dh)),
            "wo": _w((lambda *s: _rng.normal(s) * 0.05)(H * Dh, D)),
        }
    _A_in = _A_setup()

    def _B_setup():
        B, S, D, F = 1, 2048, 512, 1376
        return {
            "x": _w((lambda *s: _rng.normal(s) * 0.05)(B, S, D)),
            "w1": _w((lambda *s: _rng.normal(s) * 0.05)(D, F) * (2.0 / D) ** 0.5),
            "w3": _w((lambda *s: _rng.normal(s) * 0.05)(D, F) * (2.0 / D) ** 0.5),
            "w2": _w((lambda *s: _rng.normal(s) * 0.05)(F, D) * (2.0 / F) ** 0.5),
        }
    _B_in = _B_setup()

    return {
        "A_x": _A_in["x"],
        "A_wq": _A_in["wq"],
        "A_wk": _A_in["wk"],
        "A_wv": _A_in["wv"],
        "A_wo": _A_in["wo"],
        "B_x": _B_in["x"],
        "B_w1": _B_in["w1"],
        "B_w3": _B_in["w3"],
        "B_w2": _B_in["w2"],
    }

def _fwd_reference(A_x, A_wq, A_wk, A_wv, A_wo, B_x, B_w1, B_w3, B_w2):
    def _A_ref(x, wq, wk, wv, wo):
        B, S, D = x.shape
        H = 32
        Dh = D // H
        q = (lambda x, *d: x.transpose(*d))((x @ wq).reshape(B, S, H, Dh), 0, 2, 1, 3)
        k = x @ wk
        v = x @ wv
        scores = jnp.einsum("bhqd,bkd->bhqk", q, k) * (Dh ** -0.5)
        p = _softmax(scores, axis=-1)
        o = jnp.einsum("bhqk,bkd->bhqd", p, v)
        return (lambda x, *d: x.transpose(*d))(o, 0, 2, 1, 3).reshape(B, S, H * Dh) @ wo

    def _B_ref(x, w1, w3, w2):
        gate = jnp.einsum("bsd,df->bsf", x, w1)
        up = jnp.einsum("bsd,df->bsf", x, w3)
        h = _silu(gate) * up
        out = jnp.einsum("bsf,fd->bsd", h, w2)
        return out

    x = A_x
    h = x + _A_ref(_layernorm(x, axis=-1), A_wq, A_wk, A_wv, A_wo)
    h2 = h + _B_ref(_layernorm(h, axis=-1), B_w1, B_w3, B_w2)
    return h2


def setup_inputs():
    _inp = _fwd_setup_inputs()
    _gk = jax.random.fold_in(jax.random.key(int.from_bytes(__import__("os").urandom(4), "little")), 2**31 - 1)
    _shapes = [[1, 2048, 512]]
    _dtypes = ['bfloat16']
    _gks = jax.random.split(_gk, len(_shapes))
    _gs = [jax.random.normal(k, s, dtype=jnp.dtype(d)) * 0.05 for k, s, d in zip(_gks, _shapes, _dtypes)]
    _inp["grad_out"] = _gs[0]
    return _inp

def reference(A_x, A_wq, A_wk, A_wv, A_wo, B_w1, B_w3, B_w2, B_x, grad_out):
    _const = dict(B_x=B_x)
    def _f(*_d):
        return _fwd_reference(**{'A_x': _d[0], 'A_wq': _d[1], 'A_wk': _d[2], 'A_wv': _d[3], 'A_wo': _d[4], 'B_w1': _d[5], 'B_w3': _d[6], 'B_w2': _d[7], **_const})
    _out, _vjp = jax.vjp(_f, A_x, A_wq, A_wk, A_wv, A_wo, B_w1, B_w3, B_w2)
    _grads = _vjp(grad_out)
    _out0 = jnp.asarray(_out)
    return (_out0, *[jnp.asarray(_g) for _g in _grads])
```

```python
import functools

import jax
import jax.numpy as jnp
import jax.experimental.pallas as pl
import jax.experimental.pallas.tpu as pltpu

F32 = jnp.float32
BF16 = jnp.bfloat16

S = 2048
D = 512
H = 32
DH = 16
F = 1376
EPS = 1e-5
TQ = 128
KC = 128
NK = S // KC


def _dot(a, b):
    return jnp.dot(a, b, preferred_element_type=F32)


def _dot_nt(a, b):
    return jax.lax.dot_general(a, b, (((1,), (1,)), ((), ())), preferred_element_type=F32)


def _ln_stats_t(x):
    m = jnp.mean(x, axis=0, keepdims=True)
    xc = x - m
    var = jnp.mean(xc * xc, axis=0, keepdims=True)
    rstd = jax.lax.rsqrt(var + EPS)
    return xc * rstd, rstd


def _ln_bwd_t(dy, xhat, rstd):
    m1 = jnp.mean(dy, axis=0, keepdims=True)
    m2 = jnp.mean(dy * xhat, axis=0, keepdims=True)
    return rstd * (dy - m1 - xhat * m2)


def kernel(x_ref, g_ref,
           wq_ref, wqT_ref, wkv_ref, wkvT_ref, wo_ref, woT_ref,
           w1_ref, w1T_ref, w3_ref, w3T_ref, w2_ref, w2T_ref,
           h2_ref, dx_ref, dwq_ref, dwk_ref, dwv_ref, dwo_ref, dw1_ref, dw3_ref, dw2_ref,
           xT_s, aT_s, kT_s, vT_s, k_s, v_s,
           e_s, sc_s, q_s, o_s, do_s, dq_s, dxp_s,
           acc_wq, acc_wo, acc_w1, acc_w3, acc_w2, acc_kv):
    i = pl.program_id(0)
    nblk = pl.num_programs(0)

    @pl.when(i == 0)
    def _():
        for c in range(S // TQ):
            xt_b = x_ref[pl.ds(c * TQ, TQ), :].T
            xT_s[:, pl.ds(c * TQ, TQ)] = xt_b
            xhat, _ = _ln_stats_t(xt_b.astype(F32))
            aT_s[:, pl.ds(c * TQ, TQ)] = xhat.astype(BF16)
        kvT = _dot(wkvT_ref[...], aT_s[...]).astype(BF16)
        kT = kvT[0:DH, :]
        vT = kvT[DH:2 * DH, :]
        kT_s[...] = kT
        vT_s[...] = vT
        k_s[...] = kT.T
        v_s[...] = vT.T
        acc_wq[...] = jnp.zeros_like(acc_wq)
        acc_wo[...] = jnp.zeros_like(acc_wo)
        acc_w1[...] = jnp.zeros_like(acc_w1)
        acc_w3[...] = jnp.zeros_like(acc_w3)
        acc_w2[...] = jnp.zeros_like(acc_w2)
        acc_kv[...] = jnp.zeros_like(acc_kv)

    col0 = pl.multiple_of(i * TQ, TQ)
    aT = aT_s[:, pl.ds(col0, TQ)]
    xT = xT_s[:, pl.ds(col0, TQ)].astype(F32)

    q_s[...] = (_dot(wqT_ref[...], aT) * (DH ** -0.5)).astype(BF16)

    def fwd_head(h, carry):
        hs = pl.multiple_of(h * DH, DH)
        qh = q_s[pl.ds(hs, DH), :]
        m = jnp.full((1, TQ), -jnp.inf, F32)
        l8 = jnp.zeros((8, TQ), F32)
        o = jnp.zeros((DH, TQ), F32)
        for c in range(NK):
            ks = c * KC
            s = _dot(k_s[ks:ks + KC, :], qh)
            m_new = jnp.maximum(m, jnp.max(s, axis=0, keepdims=True))
            alpha = jnp.exp(m - m_new)
            e = jnp.exp(s - m_new)
            l8 = l8 * alpha + jnp.sum(e.reshape(KC // 8, 8, TQ), axis=0)
            eb = e.astype(BF16)
            e_s[h, ks:ks + KC, :] = eb
            o = o * alpha + _dot(vT_s[:, ks:ks + KC], eb)
            sc_s[h, c:c + 1, :] = m_new
            m = m_new
        linv = 1.0 / jnp.sum(l8, axis=0, keepdims=True)
        o_s[pl.ds(hs, DH), :] = o * linv
        sc_s[h] = jnp.exp(sc_s[h] - m) * linv
        return carry

    jax.lax.fori_loop(0, H, fwd_head, 0)

    o_f = o_s[...]
    o_b = o_f.astype(BF16)
    hT = xT + _dot(woT_ref[...], o_b)
    bT, rstd2 = _ln_stats_t(hT)
    b_b = bT.astype(BF16)
    gate = _dot(w1T_ref[...], b_b)
    up = _dot(w3T_ref[...], b_b)
    sig = jax.nn.sigmoid(gate)
    silu = gate * sig
    hh_b = (silu * up).astype(BF16)
    h2T = hT + _dot(w2T_ref[...], hh_b)
    h2_ref[...] = h2T.T.astype(BF16)

    gT = g_ref[...].T.astype(F32)
    g_b = gT.astype(BF16)
    dhh = _dot(w2_ref[...], g_b)
    acc_w2[...] += _dot_nt(hh_b, g_b)
    dgate = dhh * up * (sig * (1.0 + gate * (1.0 - sig)))
    dup = dhh * silu
    dgate_b = dgate.astype(BF16)
    dup_b = dup.astype(BF16)
    acc_w1[...] += _dot_nt(b_b, dgate_b)
    acc_w3[...] += _dot_nt(b_b, dup_b)
    dbT = _dot(w1_ref[...], dgate_b) + _dot(w3_ref[...], dup_b)
    dhT = gT + _ln_bwd_t(dbT, bT, rstd2)
    dh_b = dhT.astype(BF16)
    acc_wo[...] += _dot_nt(o_b, dh_b)
    do_s[...] = _dot(wo_ref[...], dh_b)

    def bwd_head(h, carry):
        hs = pl.multiple_of(h * DH, DH)
        do_h = do_s[pl.ds(hs, DH), :]
        o_h = o_s[pl.ds(hs, DH), :]
        dfull = jnp.sum(do_h * o_h, axis=0, keepdims=True)
        qh = q_s[pl.ds(hs, DH), :]
        sc = sc_s[h]
        dq = jnp.zeros((DH, TQ), F32)
        for c in range(NK):
            ks = c * KC
            s_c = sc[c:c + 1, :]
            dop_c = (do_h * s_c).astype(BF16)
            dp = _dot(v_s[ks:ks + KC, :], dop_c)
            eb = e_s[h, ks:ks + KC, :]
            ds = (eb.astype(F32) * (dp - dfull * s_c)).astype(BF16)
            dq = dq + _dot(kT_s[:, ks:ks + KC], ds)
            acc_kv[0:DH, ks:ks + KC] += _dot_nt(qh, ds)
            acc_kv[DH:2 * DH, ks:ks + KC] += _dot_nt(dop_c, eb)
        dq_s[pl.ds(hs, DH), :] = dq * (DH ** -0.5)
        return carry

    jax.lax.fori_loop(0, H, bwd_head, 0)

    dq_b = dq_s[...].astype(BF16)
    acc_wq[...] += _dot_nt(aT, dq_b)
    daT = _dot(wq_ref[...], dq_b)
    xhat1, rstd1 = _ln_stats_t(xT)
    dxp_s[:, pl.ds(col0, TQ)] = dhT + _ln_bwd_t(daT, xhat1, rstd1)

    @pl.when(i == nblk - 1)
    def _():
        kv_b = acc_kv[...].astype(BF16)
        dwkvT = _dot_nt(kv_b, aT_s[...])
        dwk_ref[...] = dwkvT[0:DH, :].T.astype(BF16)
        dwv_ref[...] = dwkvT[DH:2 * DH, :].T.astype(BF16)
        for c in range(S // TQ):
            cs = c * TQ
            dakv = _dot(wkv_ref[...], kv_b[:, cs:cs + TQ])
            xhat_c, rstd_c = _ln_stats_t(xT_s[:, pl.ds(cs, TQ)].astype(F32))
            dxc = dxp_s[:, pl.ds(cs, TQ)] + _ln_bwd_t(dakv, xhat_c, rstd_c)
            dx_ref[pl.ds(cs, TQ), :] = dxc.T.astype(BF16)
        dwq_ref[...] = acc_wq[...].astype(BF16)
        dwo_ref[...] = acc_wo[...].astype(BF16)
        dw1_ref[...] = acc_w1[...].astype(BF16)
        dw3_ref[...] = acc_w3[...].astype(BF16)
        dw2_ref[...] = acc_w2[...].astype(BF16)


def _full(shape):
    return pl.BlockSpec(shape, lambda i: tuple(0 for _ in shape), pipeline_mode=pl.Buffered(1))


@jax.jit
def pallas_sequential_preLN__grouped_kv_mqa__glu_gated_swiglu__prompt_kernel(
        A_x, A_wq, A_wk, A_wv, A_wo, B_x, B_w1, B_w3, B_w2, grad_out):
    x = A_x.reshape(S, D)
    g = grad_out.reshape(S, D)
    wkv = jnp.concatenate([A_wk, A_wv], axis=1)
    operands = (x, g,
                A_wq, A_wq.T, wkv, wkv.T, A_wo, A_wo.T,
                B_w1, B_w1.T, B_w3, B_w3.T, B_w2, B_w2.T)
    in_specs = [
        _full((S, D)),
        pl.BlockSpec((TQ, D), lambda i: (i, 0)),
        _full((D, D)), _full((D, D)), _full((D, 2 * DH)), _full((2 * DH, D)),
        _full((D, D)), _full((D, D)),
        _full((D, F)), _full((F, D)), _full((D, F)), _full((F, D)), _full((F, D)), _full((D, F)),
    ]
    out_shape = (
        jax.ShapeDtypeStruct((S, D), BF16),
        jax.ShapeDtypeStruct((S, D), BF16),
        jax.ShapeDtypeStruct((D, D), BF16),
        jax.ShapeDtypeStruct((D, DH), BF16),
        jax.ShapeDtypeStruct((D, DH), BF16),
        jax.ShapeDtypeStruct((D, D), BF16),
        jax.ShapeDtypeStruct((D, F), BF16),
        jax.ShapeDtypeStruct((D, F), BF16),
        jax.ShapeDtypeStruct((F, D), BF16),
    )
    out_specs = (
        pl.BlockSpec((TQ, D), lambda i: (i, 0)),
        _full((S, D)), _full((D, D)), _full((D, DH)), _full((D, DH)), _full((D, D)),
        _full((D, F)), _full((D, F)), _full((F, D)),
    )
    scratch = [
        pltpu.VMEM((D, S), BF16),
        pltpu.VMEM((D, S), BF16),
        pltpu.VMEM((DH, S), BF16),
        pltpu.VMEM((DH, S), BF16),
        pltpu.VMEM((S, DH), BF16),
        pltpu.VMEM((S, DH), BF16),
        pltpu.VMEM((H, S, TQ), BF16),
        pltpu.VMEM((H, NK, TQ), F32),
        pltpu.VMEM((D, TQ), BF16),
        pltpu.VMEM((D, TQ), F32),
        pltpu.VMEM((D, TQ), F32),
        pltpu.VMEM((D, TQ), F32),
        pltpu.VMEM((D, S), F32),
        pltpu.VMEM((D, D), F32),
        pltpu.VMEM((D, D), F32),
        pltpu.VMEM((D, F), F32),
        pltpu.VMEM((D, F), F32),
        pltpu.VMEM((F, D), F32),
        pltpu.VMEM((2 * DH, S), F32),
    ]
    outs = pl.pallas_call(
        kernel,
        grid=(S // TQ,),
        in_specs=in_specs,
        out_specs=out_specs,
        out_shape=out_shape,
        scratch_shapes=scratch,
        compiler_params=pltpu.CompilerParams(
            dimension_semantics=("arbitrary",),
            vmem_limit_bytes=110 * 1024 * 1024,
        ),
    )(*operands)
    h2, dx, dwq, dwk, dwv, dwo, dw1, dw3, dw2 = outs
    return (h2.reshape(1, S, D), dx.reshape(1, S, D), dwq, dwk, dwv, dwo, dw1, dw3, dw2)
```

```python
import functools

import jax
import jax.numpy as jnp
import jax.experimental.pallas as pl
import jax.experimental.pallas.tpu as pltpu

F32 = jnp.float32
BF16 = jnp.bfloat16

S = 2048
D = 512
H = 32
DH = 16
F = 1376
EPS = 1e-5
TQ = 256
CH = 128
NCH = S // CH


def _dot(a, b):
    return jnp.dot(a, b, preferred_element_type=F32)


def _dot_nt(a, b):
    return jax.lax.dot_general(a, b, (((1,), (1,)), ((), ())), preferred_element_type=F32)


def _ln_stats_t(x):
    m = jnp.mean(x, axis=0, keepdims=True)
    xc = x - m
    var = jnp.mean(xc * xc, axis=0, keepdims=True)
    rstd = jax.lax.rsqrt(var + EPS)
    return xc * rstd, rstd


def _ln_bwd_t(dy, xhat, rstd):
    m1 = jnp.mean(dy, axis=0, keepdims=True)
    m2 = jnp.mean(dy * xhat, axis=0, keepdims=True)
    return rstd * (dy - m1 - xhat * m2)


def kernel(x_ref, g_ref,
           wq_ref, wqT_ref, wkv_ref, wkvT_ref, wo_ref, woT_ref,
           w1_ref, w1T_ref, w3_ref, w3T_ref, w2_ref, w2T_ref,
           h2_ref, dx_ref, dwq_ref, dwk_ref, dwv_ref, dwo_ref, dw1_ref, dw3_ref, dw2_ref,
           xT_s, aT_s, kT_s, vT_s, k_s, v_s,
           e_s, linv_s, q_s, o_s, do_s, dq_s, dxp_s,
           s_a, s_b, ds_a, ds_b,
           acc_wq, acc_wo, acc_w1, acc_w3, acc_w2, acc_kv):
    i = pl.program_id(0)
    nblk = pl.num_programs(0)

    @pl.when(i == 0)
    def _():
        for c in range(S // TQ):
            xt_b = x_ref[pl.ds(c * TQ, TQ), :].T
            xT_s[:, pl.ds(c * TQ, TQ)] = xt_b
            xhat, _ = _ln_stats_t(xt_b.astype(F32))
            aT_s[:, pl.ds(c * TQ, TQ)] = xhat.astype(BF16)
        kvT = _dot(wkvT_ref[...], aT_s[...]).astype(BF16)
        kT = kvT[0:DH, :]
        vT = kvT[DH:2 * DH, :]
        kT_s[...] = kT
        vT_s[...] = vT
        k_s[...] = kT.T
        v_s[...] = vT.T
        acc_wq[...] = jnp.zeros_like(acc_wq)
        acc_wo[...] = jnp.zeros_like(acc_wo)
        acc_w1[...] = jnp.zeros_like(acc_w1)
        acc_w3[...] = jnp.zeros_like(acc_w3)
        acc_w2[...] = jnp.zeros_like(acc_w2)
        acc_kv[...] = jnp.zeros_like(acc_kv)

    col0 = pl.multiple_of(i * TQ, TQ)
    aT = aT_s[:, pl.ds(col0, TQ)]
    xT = xT_s[:, pl.ds(col0, TQ)].astype(F32)

    q_s[...] = (_dot(wqT_ref[...], aT) * (DH ** -0.5)).astype(BF16)

    def scores_into(s_ref, h):
        hs = pl.multiple_of(h * DH, DH)
        s_ref[...] = _dot(k_s[...], q_s[pl.ds(hs, DH), :])

    def softmax_head(s_ref, h):
        hs = pl.multiple_of(h * DH, DH)
        m8 = jnp.max(s_ref[...].reshape(S // 8, 8, TQ), axis=0)
        m = jnp.max(m8, axis=0, keepdims=True)
        l8 = jnp.zeros((8, TQ), F32)
        for c in range(NCH):
            cs = c * CH
            e = jnp.exp(s_ref[cs:cs + CH, :] - m)
            l8 = l8 + jnp.sum(e.reshape(CH // 8, 8, TQ), axis=0)
            e_s[h, cs:cs + CH, :] = e.astype(BF16)
        linv = 1.0 / jnp.sum(l8, axis=0, keepdims=True)
        linv_s[h] = linv
        o_s[pl.ds(hs, DH), :] = _dot(vT_s[...], e_s[h]) * linv

    def fwd_pair(j, carry):
        h_a = 2 * j
        h_b = 2 * j + 1
        scores_into(s_b, h_b)
        softmax_head(s_a, h_a)
        scores_into(s_a, jnp.minimum(h_a + 2, H - 1))
        softmax_head(s_b, h_b)
        return carry

    scores_into(s_a, jnp.int32(0))
    jax.lax.fori_loop(0, H // 2, fwd_pair, 0)

    o_f = o_s[...]
    o_b = o_f.astype(BF16)
    hT = xT + _dot(woT_ref[...], o_b)
    bT, rstd2 = _ln_stats_t(hT)
    b_b = bT.astype(BF16)
    gate = _dot(w1T_ref[...], b_b)
    up = _dot(w3T_ref[...], b_b)
    sig = jax.nn.sigmoid(gate)
    silu = gate * sig
    hh_b = (silu * up).astype(BF16)
    h2T = hT + _dot(w2T_ref[...], hh_b)
    h2_ref[...] = h2T.T.astype(BF16)

    gT = g_ref[...].T.astype(F32)
    g_b = gT.astype(BF16)
    dhh = _dot(w2_ref[...], g_b)
    acc_w2[...] += _dot_nt(hh_b, g_b)
    dgate = dhh * up * (sig * (1.0 + gate * (1.0 - sig)))
    dup = dhh * silu
    dgate_b = dgate.astype(BF16)
    dup_b = dup.astype(BF16)
    acc_w1[...] += _dot_nt(b_b, dgate_b)
    acc_w3[...] += _dot_nt(b_b, dup_b)
    dbT = _dot(w1_ref[...], dgate_b) + _dot(w3_ref[...], dup_b)
    dhT = gT + _ln_bwd_t(dbT, bT, rstd2)
    dh_b = dhT.astype(BF16)
    acc_wo[...] += _dot_nt(o_b, dh_b)
    do_s[...] = _dot(wo_ref[...], dh_b)

    def dp_into(s_ref, h):
        hs = pl.multiple_of(h * DH, DH)
        dop = (do_s[pl.ds(hs, DH), :] * linv_s[h]).astype(BF16)
        s_ref[...] = _dot(v_s[...], dop)

    def ds_from(s_ref, ds_ref, h):
        hs = pl.multiple_of(h * DH, DH)
        dop = do_s[pl.ds(hs, DH), :] * linv_s[h]
        dpr = jnp.sum(dop * o_s[pl.ds(hs, DH), :], axis=0, keepdims=True)
        for c in range(NCH):
            cs = c * CH
            ds_ref[cs:cs + CH, :] = (e_s[h, cs:cs + CH, :].astype(F32)
                                     * (s_ref[cs:cs + CH, :] - dpr)).astype(BF16)

    def mm_head(ds_ref, h):
        hs = pl.multiple_of(h * DH, DH)
        dop_b = (do_s[pl.ds(hs, DH), :] * linv_s[h]).astype(BF16)
        dq_s[pl.ds(hs, DH), :] = _dot(kT_s[...], ds_ref[...]) * (DH ** -0.5)
        acc_kv[0:DH, :] += _dot_nt(q_s[pl.ds(hs, DH), :], ds_ref[...])
        acc_kv[DH:2 * DH, :] += _dot_nt(dop_b, e_s[h])

    def bwd_pair(j, carry):
        h_a = 2 * j
        h_b = 2 * j + 1
        dp_into(s_b, h_b)
        ds_from(s_a, ds_a, h_a)
        mm_head(ds_a, h_a)
        dp_into(s_a, jnp.minimum(h_a + 2, H - 1))
        ds_from(s_b, ds_b, h_b)
        mm_head(ds_b, h_b)
        return carry

    dp_into(s_a, jnp.int32(0))
    jax.lax.fori_loop(0, H // 2, bwd_pair, 0)

    dq_b = dq_s[...].astype(BF16)
    acc_wq[...] += _dot_nt(aT, dq_b)
    daT = _dot(wq_ref[...], dq_b)
    xhat1, rstd1 = _ln_stats_t(xT)
    dxp_s[:, pl.ds(col0, TQ)] = dhT + _ln_bwd_t(daT, xhat1, rstd1)

    @pl.when(i == nblk - 1)
    def _():
        kv_b = acc_kv[...].astype(BF16)
        dwkvT = _dot_nt(kv_b, aT_s[...])
        dwk_ref[...] = dwkvT[0:DH, :].T.astype(BF16)
        dwv_ref[...] = dwkvT[DH:2 * DH, :].T.astype(BF16)
        for c in range(S // TQ):
            cs = c * TQ
            dakv = _dot(wkv_ref[...], kv_b[:, cs:cs + TQ])
            xhat_c, rstd_c = _ln_stats_t(xT_s[:, pl.ds(cs, TQ)].astype(F32))
            dxc = dxp_s[:, pl.ds(cs, TQ)] + _ln_bwd_t(dakv, xhat_c, rstd_c)
            dx_ref[pl.ds(cs, TQ), :] = dxc.T.astype(BF16)
        dwq_ref[...] = acc_wq[...].astype(BF16)
        dwo_ref[...] = acc_wo[...].astype(BF16)
        dw1_ref[...] = acc_w1[...].astype(BF16)
        dw3_ref[...] = acc_w3[...].astype(BF16)
        dw2_ref[...] = acc_w2[...].astype(BF16)


def _full(shape):
    return pl.BlockSpec(shape, lambda i: tuple(0 for _ in shape), pipeline_mode=pl.Buffered(1))


@jax.jit
def pallas_sequential_preLN__grouped_kv_mqa__glu_gated_swiglu__prompt_kernel(
        A_x, A_wq, A_wk, A_wv, A_wo, B_x, B_w1, B_w3, B_w2, grad_out):
    x = A_x.reshape(S, D)
    g = grad_out.reshape(S, D)
    wkv = jnp.concatenate([A_wk, A_wv], axis=1)
    operands = (x, g,
                A_wq, A_wq.T, wkv, wkv.T, A_wo, A_wo.T,
                B_w1, B_w1.T, B_w3, B_w3.T, B_w2, B_w2.T)
    in_specs = [
        _full((S, D)),
        pl.BlockSpec((TQ, D), lambda i: (i, 0)),
        _full((D, D)), _full((D, D)), _full((D, 2 * DH)), _full((2 * DH, D)),
        _full((D, D)), _full((D, D)),
        _full((D, F)), _full((F, D)), _full((D, F)), _full((F, D)), _full((F, D)), _full((D, F)),
    ]
    out_shape = (
        jax.ShapeDtypeStruct((S, D), BF16),
        jax.ShapeDtypeStruct((S, D), BF16),
        jax.ShapeDtypeStruct((D, D), BF16),
        jax.ShapeDtypeStruct((D, DH), BF16),
        jax.ShapeDtypeStruct((D, DH), BF16),
        jax.ShapeDtypeStruct((D, D), BF16),
        jax.ShapeDtypeStruct((D, F), BF16),
        jax.ShapeDtypeStruct((D, F), BF16),
        jax.ShapeDtypeStruct((F, D), BF16),
    )
    out_specs = (
        pl.BlockSpec((TQ, D), lambda i: (i, 0)),
        _full((S, D)), _full((D, D)), _full((D, DH)), _full((D, DH)), _full((D, D)),
        _full((D, F)), _full((D, F)), _full((F, D)),
    )
    scratch = [
        pltpu.VMEM((D, S), BF16),
        pltpu.VMEM((D, S), BF16),
        pltpu.VMEM((DH, S), BF16),
        pltpu.VMEM((DH, S), BF16),
        pltpu.VMEM((S, DH), BF16),
        pltpu.VMEM((S, DH), BF16),
        pltpu.VMEM((H, S, TQ), BF16),
        pltpu.VMEM((H, 1, TQ), F32),
        pltpu.VMEM((D, TQ), BF16),
        pltpu.VMEM((D, TQ), F32),
        pltpu.VMEM((D, TQ), F32),
        pltpu.VMEM((D, TQ), F32),
        pltpu.VMEM((D, S), F32),
        pltpu.VMEM((S, TQ), F32),
        pltpu.VMEM((S, TQ), F32),
        pltpu.VMEM((S, TQ), BF16),
        pltpu.VMEM((S, TQ), BF16),
        pltpu.VMEM((D, D), F32),
        pltpu.VMEM((D, D), F32),
        pltpu.VMEM((D, F), F32),
        pltpu.VMEM((D, F), F32),
        pltpu.VMEM((F, D), F32),
        pltpu.VMEM((2 * DH, S), F32),
    ]
    outs = pl.pallas_call(
        kernel,
        grid=(S // TQ,),
        in_specs=in_specs,
        out_specs=out_specs,
        out_shape=out_shape,
        scratch_shapes=scratch,
        compiler_params=pltpu.CompilerParams(
            dimension_semantics=("arbitrary",),
            vmem_limit_bytes=110 * 1024 * 1024,
        ),
    )(*operands)
    h2, dx, dwq, dwk, dwv, dwo, dw1, dw3, dw2 = outs
    return (h2.reshape(1, S, D), dx.reshape(1, S, D), dwq, dwk, dwv, dwo, dw1, dw3, dw2)
```

```python
import functools

import jax
import jax.numpy as jnp
import jax.experimental.pallas as pl
import jax.experimental.pallas.tpu as pltpu

F32 = jnp.float32
BF16 = jnp.bfloat16

S = 2048
D = 512
H = 32
DH = 16
F = 1376
EPS = 1e-5
TQ = 256
CH = 128
NCH = S // CH


def _dot(a, b):
    return jnp.dot(a, b, preferred_element_type=F32)


def _dot_nt(a, b):
    return jax.lax.dot_general(a, b, (((1,), (1,)), ((), ())), preferred_element_type=F32)


def _ln_stats_t(x):
    m = jnp.mean(x, axis=0, keepdims=True)
    xc = x - m
    var = jnp.mean(xc * xc, axis=0, keepdims=True)
    rstd = jax.lax.rsqrt(var + EPS)
    return xc * rstd, rstd


def _ln_bwd_t(dy, xhat, rstd):
    m1 = jnp.mean(dy, axis=0, keepdims=True)
    m2 = jnp.mean(dy * xhat, axis=0, keepdims=True)
    return rstd * (dy - m1 - xhat * m2)


def kernel(x_ref, g_ref,
           wq_ref, wqT_ref, wkv_ref, wkvT_ref, wo_ref, woT_ref,
           w1_ref, w1T_ref, w3_ref, w3T_ref, w2_ref, w2T_ref,
           h2_ref, dx_ref, dwq_ref, dwk_ref, dwv_ref, dwo_ref, dw1_ref, dw3_ref, dw2_ref,
           xT_s, aT_s, kT_s, vT_s, k_s, v_s,
           e_s, linv_s, q_s, o_s, do_s, dq_s, dxp_s,
           s_a, s_b, ds_a, ds_b,
           acc_wq, acc_wo, acc_w1, acc_w3, acc_w2, acc_kv):
    i = pl.program_id(0)
    nblk = pl.num_programs(0)

    @pl.when(i == 0)
    def _():
        for c in range(S // TQ):
            xt_b = x_ref[pl.ds(c * TQ, TQ), :].T
            xT_s[:, pl.ds(c * TQ, TQ)] = xt_b
            xhat, _ = _ln_stats_t(xt_b.astype(F32))
            aT_s[:, pl.ds(c * TQ, TQ)] = xhat.astype(BF16)
        kvT = _dot(wkvT_ref[...], aT_s[...]).astype(BF16)
        kT = kvT[0:DH, :]
        vT = kvT[DH:2 * DH, :]
        kT_s[...] = kT
        vT_s[...] = vT
        k_s[...] = kT.T
        v_s[...] = vT.T
        acc_wq[...] = jnp.zeros_like(acc_wq)
        acc_wo[...] = jnp.zeros_like(acc_wo)
        acc_w1[...] = jnp.zeros_like(acc_w1)
        acc_w3[...] = jnp.zeros_like(acc_w3)
        acc_w2[...] = jnp.zeros_like(acc_w2)
        acc_kv[...] = jnp.zeros_like(acc_kv)

    col0 = pl.multiple_of(i * TQ, TQ)
    aT = aT_s[:, pl.ds(col0, TQ)]
    xT = xT_s[:, pl.ds(col0, TQ)].astype(F32)

    q_s[...] = (_dot(wqT_ref[...], aT) * (DH ** -0.5)).astype(BF16)

    def scores_into(s_ref, h):
        hs = pl.multiple_of(h * DH, DH)
        s_ref[...] = _dot(k_s[...], q_s[pl.ds(hs, DH), :])

    def softmax_head(s_ref, h):
        hs = pl.multiple_of(h * DH, DH)
        m8 = jnp.max(s_ref[...].reshape(S // 8, 8, TQ), axis=0)
        m = jnp.max(m8, axis=0, keepdims=True)
        mb = jnp.broadcast_to(m, (8, TQ))
        l8 = jnp.zeros((8, TQ), F32)
        for c in range(NCH):
            cs = c * CH
            sc = s_ref[cs:cs + CH, :].reshape(CH // 8, 8, TQ)
            e = jnp.exp(sc - mb[None])
            l8 = l8 + jnp.sum(e, axis=0)
            e_s[h, cs:cs + CH, :] = e.reshape(CH, TQ).astype(BF16)
        linv = 1.0 / jnp.sum(l8, axis=0, keepdims=True)
        linv_s[h] = linv
        o_s[pl.ds(hs, DH), :] = _dot(vT_s[...], e_s[h]) * linv

    def fwd_pair(j, carry):
        h_a = 2 * j
        h_b = 2 * j + 1
        scores_into(s_b, h_b)
        softmax_head(s_a, h_a)
        scores_into(s_a, jnp.minimum(h_a + 2, H - 1))
        softmax_head(s_b, h_b)
        return carry

    scores_into(s_a, jnp.int32(0))
    jax.lax.fori_loop(0, H // 2, fwd_pair, 0)

    o_f = o_s[...]
    o_b = o_f.astype(BF16)
    hT = xT + _dot(woT_ref[...], o_b)
    bT, rstd2 = _ln_stats_t(hT)
    b_b = bT.astype(BF16)
    gate = _dot(w1T_ref[...], b_b)
    up = _dot(w3T_ref[...], b_b)
    sig = jax.nn.sigmoid(gate)
    silu = gate * sig
    hh_b = (silu * up).astype(BF16)
    h2T = hT + _dot(w2T_ref[...], hh_b)
    h2_ref[...] = h2T.T.astype(BF16)

    gT = g_ref[...].T.astype(F32)
    g_b = gT.astype(BF16)
    dhh = _dot(w2_ref[...], g_b)
    acc_w2[...] += _dot_nt(hh_b, g_b)
    dgate = dhh * up * (sig * (1.0 + gate * (1.0 - sig)))
    dup = dhh * silu
    dgate_b = dgate.astype(BF16)
    dup_b = dup.astype(BF16)
    acc_w1[...] += _dot_nt(b_b, dgate_b)
    acc_w3[...] += _dot_nt(b_b, dup_b)
    dbT = _dot(w1_ref[...], dgate_b) + _dot(w3_ref[...], dup_b)
    dhT = gT + _ln_bwd_t(dbT, bT, rstd2)
    dh_b = dhT.astype(BF16)
    acc_wo[...] += _dot_nt(o_b, dh_b)
    do_s[...] = _dot(wo_ref[...], dh_b)

    def dp_into(s_ref, h):
        hs = pl.multiple_of(h * DH, DH)
        dop = (do_s[pl.ds(hs, DH), :] * linv_s[h]).astype(BF16)
        s_ref[...] = _dot(v_s[...], dop)

    def ds_from(s_ref, ds_ref, h):
        hs = pl.multiple_of(h * DH, DH)
        dop = do_s[pl.ds(hs, DH), :] * linv_s[h]
        dpr = jnp.sum(dop * o_s[pl.ds(hs, DH), :], axis=0, keepdims=True)
        dprb = jnp.broadcast_to(dpr, (8, TQ))
        for c in range(NCH):
            cs = c * CH
            dpc = s_ref[cs:cs + CH, :].reshape(CH // 8, 8, TQ) - dprb[None]
            ec = e_s[h, cs:cs + CH, :].astype(F32).reshape(CH // 8, 8, TQ)
            ds_ref[cs:cs + CH, :] = (ec * dpc).reshape(CH, TQ).astype(BF16)

    def mm_head(ds_ref, h):
        hs = pl.multiple_of(h * DH, DH)
        dop_b = (do_s[pl.ds(hs, DH), :] * linv_s[h]).astype(BF16)
        dq_s[pl.ds(hs, DH), :] = _dot(kT_s[...], ds_ref[...]) * (DH ** -0.5)
        acc_kv[0:DH, :] += _dot_nt(q_s[pl.ds(hs, DH), :], ds_ref[...])
        acc_kv[DH:2 * DH, :] += _dot_nt(dop_b, e_s[h])

    def bwd_pair(j, carry):
        h_a = 2 * j
        h_b = 2 * j + 1
        dp_into(s_b, h_b)
        ds_from(s_a, ds_a, h_a)
        mm_head(ds_a, h_a)
        dp_into(s_a, jnp.minimum(h_a + 2, H - 1))
        ds_from(s_b, ds_b, h_b)
        mm_head(ds_b, h_b)
        return carry

    dp_into(s_a, jnp.int32(0))
    jax.lax.fori_loop(0, H // 2, bwd_pair, 0)

    dq_b = dq_s[...].astype(BF16)
    acc_wq[...] += _dot_nt(aT, dq_b)
    daT = _dot(wq_ref[...], dq_b)
    xhat1, rstd1 = _ln_stats_t(xT)
    dxp_s[:, pl.ds(col0, TQ)] = dhT + _ln_bwd_t(daT, xhat1, rstd1)

    @pl.when(i == nblk - 1)
    def _():
        kv_b = acc_kv[...].astype(BF16)
        dwkvT = _dot_nt(kv_b, aT_s[...])
        dwk_ref[...] = dwkvT[0:DH, :].T.astype(BF16)
        dwv_ref[...] = dwkvT[DH:2 * DH, :].T.astype(BF16)
        for c in range(S // TQ):
            cs = c * TQ
            dakv = _dot(wkv_ref[...], kv_b[:, cs:cs + TQ])
            xhat_c, rstd_c = _ln_stats_t(xT_s[:, pl.ds(cs, TQ)].astype(F32))
            dxc = dxp_s[:, pl.ds(cs, TQ)] + _ln_bwd_t(dakv, xhat_c, rstd_c)
            dx_ref[pl.ds(cs, TQ), :] = dxc.T.astype(BF16)
        dwq_ref[...] = acc_wq[...].astype(BF16)
        dwo_ref[...] = acc_wo[...].astype(BF16)
        dw1_ref[...] = acc_w1[...].astype(BF16)
        dw3_ref[...] = acc_w3[...].astype(BF16)
        dw2_ref[...] = acc_w2[...].astype(BF16)


def _full(shape):
    return pl.BlockSpec(shape, lambda i: tuple(0 for _ in shape), pipeline_mode=pl.Buffered(1))


@jax.jit
def pallas_sequential_preLN__grouped_kv_mqa__glu_gated_swiglu__prompt_kernel(
        A_x, A_wq, A_wk, A_wv, A_wo, B_x, B_w1, B_w3, B_w2, grad_out):
    x = A_x.reshape(S, D)
    g = grad_out.reshape(S, D)
    wkv = jnp.concatenate([A_wk, A_wv], axis=1)
    operands = (x, g,
                A_wq, A_wq.T, wkv, wkv.T, A_wo, A_wo.T,
                B_w1, B_w1.T, B_w3, B_w3.T, B_w2, B_w2.T)
    in_specs = [
        _full((S, D)),
        pl.BlockSpec((TQ, D), lambda i: (i, 0)),
        _full((D, D)), _full((D, D)), _full((D, 2 * DH)), _full((2 * DH, D)),
        _full((D, D)), _full((D, D)),
        _full((D, F)), _full((F, D)), _full((D, F)), _full((F, D)), _full((F, D)), _full((D, F)),
    ]
    out_shape = (
        jax.ShapeDtypeStruct((S, D), BF16),
        jax.ShapeDtypeStruct((S, D), BF16),
        jax.ShapeDtypeStruct((D, D), BF16),
        jax.ShapeDtypeStruct((D, DH), BF16),
        jax.ShapeDtypeStruct((D, DH), BF16),
        jax.ShapeDtypeStruct((D, D), BF16),
        jax.ShapeDtypeStruct((D, F), BF16),
        jax.ShapeDtypeStruct((D, F), BF16),
        jax.ShapeDtypeStruct((F, D), BF16),
    )
    out_specs = (
        pl.BlockSpec((TQ, D), lambda i: (i, 0)),
        _full((S, D)), _full((D, D)), _full((D, DH)), _full((D, DH)), _full((D, D)),
        _full((D, F)), _full((D, F)), _full((F, D)),
    )
    scratch = [
        pltpu.VMEM((D, S), BF16),
        pltpu.VMEM((D, S), BF16),
        pltpu.VMEM((DH, S), BF16),
        pltpu.VMEM((DH, S), BF16),
        pltpu.VMEM((S, DH), BF16),
        pltpu.VMEM((S, DH), BF16),
        pltpu.VMEM((H, S, TQ), BF16),
        pltpu.VMEM((H, 1, TQ), F32),
        pltpu.VMEM((D, TQ), BF16),
        pltpu.VMEM((D, TQ), F32),
        pltpu.VMEM((D, TQ), F32),
        pltpu.VMEM((D, TQ), F32),
        pltpu.VMEM((D, S), F32),
        pltpu.VMEM((S, TQ), F32),
        pltpu.VMEM((S, TQ), F32),
        pltpu.VMEM((S, TQ), BF16),
        pltpu.VMEM((S, TQ), BF16),
        pltpu.VMEM((D, D), F32),
        pltpu.VMEM((D, D), F32),
        pltpu.VMEM((D, F), F32),
        pltpu.VMEM((D, F), F32),
        pltpu.VMEM((F, D), F32),
        pltpu.VMEM((2 * DH, S), F32),
    ]
    outs = pl.pallas_call(
        kernel,
        grid=(S // TQ,),
        in_specs=in_specs,
        out_specs=out_specs,
        out_shape=out_shape,
        scratch_shapes=scratch,
        compiler_params=pltpu.CompilerParams(
            dimension_semantics=("arbitrary",),
            vmem_limit_bytes=110 * 1024 * 1024,
        ),
    )(*operands)
    h2, dx, dwq, dwk, dwv, dwo, dw1, dw3, dw2 = outs
    return (h2.reshape(1, S, D), dx.reshape(1, S, D), dwq, dwk, dwv, dwo, dw1, dw3, dw2)
```

```python
import functools

import jax
import jax.numpy as jnp
import jax.experimental.pallas as pl
import jax.experimental.pallas.tpu as pltpu

F32 = jnp.float32
BF16 = jnp.bfloat16

S = 2048
D = 512
H = 32
DH = 16
F = 1376
EPS = 1e-5
TQ = 256
TG = 2 * TQ
CH = 64
NCH = S // CH


def _dot(a, b):
    return jnp.dot(a, b, preferred_element_type=F32)


def _dot_nt(a, b):
    return jax.lax.dot_general(a, b, (((1,), (1,)), ((), ())), preferred_element_type=F32)


def _ln_stats_t(x):
    m = jnp.mean(x, axis=0, keepdims=True)
    xc = x - m
    var = jnp.mean(xc * xc, axis=0, keepdims=True)
    rstd = jax.lax.rsqrt(var + EPS)
    return xc * rstd, rstd


def _ln_bwd_t(dy, xhat, rstd):
    m1 = jnp.mean(dy, axis=0, keepdims=True)
    m2 = jnp.mean(dy * xhat, axis=0, keepdims=True)
    return rstd * (dy - m1 - xhat * m2)


def kernel(x_ref, g_ref,
           wq_ref, wqT_ref, wkv_ref, wkvT_ref, wo_ref, woT_ref,
           w1_ref, w1T_ref, w3_ref, w3T_ref, w2_ref, w2T_ref,
           h2_ref, dx_ref, dwq_ref, dwk_ref, dwv_ref, dwo_ref, dw1_ref, dw3_ref, dw2_ref,
           xT_s, aT_s, kT_s, vT_s, k_s, v_s,
           e_s, linv_s, q_s, o_s, do_s, dq_s, dxp_s,
           s_a, s_b, ds_a, ds_b,
           acc_wq, acc_wo, acc_w1, acc_w3, acc_w2, acc_kv):
    i = pl.program_id(0)
    nblk = pl.num_programs(0)

    @pl.when(i == 0)
    def _():
        for c in range(S // TQ):
            xt_b = x_ref[pl.ds(c * TQ, TQ), :].T
            xT_s[:, pl.ds(c * TQ, TQ)] = xt_b
            xhat, _ = _ln_stats_t(xt_b.astype(F32))
            aT_s[:, pl.ds(c * TQ, TQ)] = xhat.astype(BF16)
        kvT = _dot(wkvT_ref[...], aT_s[...]).astype(BF16)
        kT = kvT[0:DH, :]
        vT = kvT[DH:2 * DH, :]
        kT_s[...] = kT
        vT_s[...] = vT
        k_s[...] = kT.T
        v_s[...] = vT.T
        acc_wq[...] = jnp.zeros_like(acc_wq)
        acc_wo[...] = jnp.zeros_like(acc_wo)
        acc_w1[...] = jnp.zeros_like(acc_w1)
        acc_w3[...] = jnp.zeros_like(acc_w3)
        acc_w2[...] = jnp.zeros_like(acc_w2)
        acc_kv[...] = jnp.zeros_like(acc_kv)

    col0 = pl.multiple_of(i * TQ, TQ)
    aT = aT_s[:, pl.ds(col0, TQ)]
    xT = xT_s[:, pl.ds(col0, TQ)].astype(F32)

    q_s[...] = (_dot(wqT_ref[...], aT) * (DH ** -0.5)).astype(BF16)

    def scores_group(s_ref, j):
        h_a = 2 * j
        hsa = pl.multiple_of(h_a * DH, DH)
        hsb = pl.multiple_of((h_a + 1) * DH, DH)
        qg = jnp.concatenate([q_s[pl.ds(hsa, DH), :], q_s[pl.ds(hsb, DH), :]], axis=1)
        s_ref[...] = _dot(k_s[...], qg)

    def softmax_head(s_ref, off, h):
        hs = pl.multiple_of(h * DH, DH)
        m8 = jnp.max(s_ref[:, off:off + TQ].reshape(S // 8, 8, TQ), axis=0)
        m = jnp.max(m8, axis=0, keepdims=True)
        mb = jnp.broadcast_to(m, (8, TQ))
        l8 = jnp.zeros((8, TQ), F32)
        for c in range(NCH):
            cs = c * CH
            sc = s_ref[cs:cs + CH, off:off + TQ].reshape(CH // 8, 8, TQ)
            e = jnp.exp(sc - mb[None])
            l8 = l8 + jnp.sum(e, axis=0)
            e_s[h, cs:cs + CH, :] = e.reshape(CH, TQ).astype(BF16)
        linv = 1.0 / jnp.sum(l8, axis=0, keepdims=True)
        linv_s[h] = linv
        o_s[pl.ds(hs, DH), :] = _dot(vT_s[...], e_s[h]) * linv

    def fwd_quad(i, carry):
        ja = 2 * i
        jb = 2 * i + 1
        scores_group(s_b, jb)
        softmax_head(s_a, 0, 2 * ja)
        softmax_head(s_a, TQ, 2 * ja + 1)
        scores_group(s_a, jnp.minimum(ja + 2, H // 2 - 1))
        softmax_head(s_b, 0, 2 * jb)
        softmax_head(s_b, TQ, 2 * jb + 1)
        return carry

    scores_group(s_a, jnp.int32(0))
    jax.lax.fori_loop(0, H // 4, fwd_quad, 0)

    o_f = o_s[...]
    o_b = o_f.astype(BF16)
    hT = xT + _dot(woT_ref[...], o_b)
    bT, rstd2 = _ln_stats_t(hT)
    b_b = bT.astype(BF16)
    gate = _dot(w1T_ref[...], b_b)
    up = _dot(w3T_ref[...], b_b)
    sig = jax.nn.sigmoid(gate)
    silu = gate * sig
    hh_b = (silu * up).astype(BF16)
    h2T = hT + _dot(w2T_ref[...], hh_b)
    h2_ref[...] = h2T.T.astype(BF16)

    gT = g_ref[...].T.astype(F32)
    g_b = gT.astype(BF16)
    dhh = _dot(w2_ref[...], g_b)
    acc_w2[...] += _dot_nt(hh_b, g_b)
    dgate = dhh * up * (sig * (1.0 + gate * (1.0 - sig)))
    dup = dhh * silu
    dgate_b = dgate.astype(BF16)
    dup_b = dup.astype(BF16)
    acc_w1[...] += _dot_nt(b_b, dgate_b)
    acc_w3[...] += _dot_nt(b_b, dup_b)
    dbT = _dot(w1_ref[...], dgate_b) + _dot(w3_ref[...], dup_b)
    dhT = gT + _ln_bwd_t(dbT, bT, rstd2)
    dh_b = dhT.astype(BF16)
    acc_wo[...] += _dot_nt(o_b, dh_b)
    do_s[...] = _dot(wo_ref[...], dh_b)

    def dp_group(s_ref, j):
        h_a = 2 * j
        hsa = pl.multiple_of(h_a * DH, DH)
        hsb = pl.multiple_of((h_a + 1) * DH, DH)
        dopa = (do_s[pl.ds(hsa, DH), :] * linv_s[h_a]).astype(BF16)
        dopb = (do_s[pl.ds(hsb, DH), :] * linv_s[h_a + 1]).astype(BF16)
        s_ref[...] = _dot(v_s[...], jnp.concatenate([dopa, dopb], axis=1))

    def ds_from(s_ref, off, ds_ref, h):
        hs = pl.multiple_of(h * DH, DH)
        dop = do_s[pl.ds(hs, DH), :] * linv_s[h]
        dpr = jnp.sum(dop * o_s[pl.ds(hs, DH), :], axis=0, keepdims=True)
        dprb = jnp.broadcast_to(dpr, (8, TQ))
        for c in range(NCH):
            cs = c * CH
            dpc = s_ref[cs:cs + CH, off:off + TQ].reshape(CH // 8, 8, TQ) - dprb[None]
            ec = e_s[h, cs:cs + CH, :].astype(F32).reshape(CH // 8, 8, TQ)
            ds_ref[cs:cs + CH, :] = (ec * dpc).reshape(CH, TQ).astype(BF16)

    def mm_head(ds_ref, h):
        hs = pl.multiple_of(h * DH, DH)
        dop_b = (do_s[pl.ds(hs, DH), :] * linv_s[h]).astype(BF16)
        dq_s[pl.ds(hs, DH), :] = _dot(kT_s[...], ds_ref[...]) * (DH ** -0.5)
        acc_kv[0:DH, :] += _dot_nt(q_s[pl.ds(hs, DH), :], ds_ref[...])
        acc_kv[DH:2 * DH, :] += _dot_nt(dop_b, e_s[h])

    def bwd_quad(i, carry):
        ja = 2 * i
        jb = 2 * i + 1
        dp_group(s_b, jb)
        ds_from(s_a, 0, ds_a, 2 * ja)
        mm_head(ds_a, 2 * ja)
        ds_from(s_a, TQ, ds_a, 2 * ja + 1)
        mm_head(ds_a, 2 * ja + 1)
        dp_group(s_a, jnp.minimum(ja + 2, H // 2 - 1))
        ds_from(s_b, 0, ds_b, 2 * jb)
        mm_head(ds_b, 2 * jb)
        ds_from(s_b, TQ, ds_b, 2 * jb + 1)
        mm_head(ds_b, 2 * jb + 1)
        return carry

    dp_group(s_a, jnp.int32(0))
    jax.lax.fori_loop(0, H // 4, bwd_quad, 0)

    dq_b = dq_s[...].astype(BF16)
    acc_wq[...] += _dot_nt(aT, dq_b)
    daT = _dot(wq_ref[...], dq_b)
    xhat1, rstd1 = _ln_stats_t(xT)
    dxp_s[:, pl.ds(col0, TQ)] = dhT + _ln_bwd_t(daT, xhat1, rstd1)

    @pl.when(i == nblk - 1)
    def _():
        kv_b = acc_kv[...].astype(BF16)
        dwkvT = _dot_nt(kv_b, aT_s[...])
        dwk_ref[...] = dwkvT[0:DH, :].T.astype(BF16)
        dwv_ref[...] = dwkvT[DH:2 * DH, :].T.astype(BF16)
        for c in range(S // TQ):
            cs = c * TQ
            dakv = _dot(wkv_ref[...], kv_b[:, cs:cs + TQ])
            xhat_c, rstd_c = _ln_stats_t(xT_s[:, pl.ds(cs, TQ)].astype(F32))
            dxc = dxp_s[:, pl.ds(cs, TQ)] + _ln_bwd_t(dakv, xhat_c, rstd_c)
            dx_ref[pl.ds(cs, TQ), :] = dxc.T.astype(BF16)
        dwq_ref[...] = acc_wq[...].astype(BF16)
        dwo_ref[...] = acc_wo[...].astype(BF16)
        dw1_ref[...] = acc_w1[...].astype(BF16)
        dw3_ref[...] = acc_w3[...].astype(BF16)
        dw2_ref[...] = acc_w2[...].astype(BF16)


def _full(shape):
    return pl.BlockSpec(shape, lambda i: tuple(0 for _ in shape), pipeline_mode=pl.Buffered(1))


@jax.jit
def pallas_sequential_preLN__grouped_kv_mqa__glu_gated_swiglu__prompt_kernel(
        A_x, A_wq, A_wk, A_wv, A_wo, B_x, B_w1, B_w3, B_w2, grad_out):
    x = A_x.reshape(S, D)
    g = grad_out.reshape(S, D)
    wkv = jnp.concatenate([A_wk, A_wv], axis=1)
    operands = (x, g,
                A_wq, A_wq.T, wkv, wkv.T, A_wo, A_wo.T,
                B_w1, B_w1.T, B_w3, B_w3.T, B_w2, B_w2.T)
    in_specs = [
        _full((S, D)),
        pl.BlockSpec((TQ, D), lambda i: (i, 0)),
        _full((D, D)), _full((D, D)), _full((D, 2 * DH)), _full((2 * DH, D)),
        _full((D, D)), _full((D, D)),
        _full((D, F)), _full((F, D)), _full((D, F)), _full((F, D)), _full((F, D)), _full((D, F)),
    ]
    out_shape = (
        jax.ShapeDtypeStruct((S, D), BF16),
        jax.ShapeDtypeStruct((S, D), BF16),
        jax.ShapeDtypeStruct((D, D), BF16),
        jax.ShapeDtypeStruct((D, DH), BF16),
        jax.ShapeDtypeStruct((D, DH), BF16),
        jax.ShapeDtypeStruct((D, D), BF16),
        jax.ShapeDtypeStruct((D, F), BF16),
        jax.ShapeDtypeStruct((D, F), BF16),
        jax.ShapeDtypeStruct((F, D), BF16),
    )
    out_specs = (
        pl.BlockSpec((TQ, D), lambda i: (i, 0)),
        _full((S, D)), _full((D, D)), _full((D, DH)), _full((D, DH)), _full((D, D)),
        _full((D, F)), _full((D, F)), _full((F, D)),
    )
    scratch = [
        pltpu.VMEM((D, S), BF16),
        pltpu.VMEM((D, S), BF16),
        pltpu.VMEM((DH, S), BF16),
        pltpu.VMEM((DH, S), BF16),
        pltpu.VMEM((S, DH), BF16),
        pltpu.VMEM((S, DH), BF16),
        pltpu.VMEM((H, S, TQ), BF16),
        pltpu.VMEM((H, 1, TQ), F32),
        pltpu.VMEM((D, TQ), BF16),
        pltpu.VMEM((D, TQ), F32),
        pltpu.VMEM((D, TQ), F32),
        pltpu.VMEM((D, TQ), F32),
        pltpu.VMEM((D, S), F32),
        pltpu.VMEM((S, TG), F32),
        pltpu.VMEM((S, TG), F32),
        pltpu.VMEM((S, TQ), BF16),
        pltpu.VMEM((S, TQ), BF16),
        pltpu.VMEM((D, D), F32),
        pltpu.VMEM((D, D), F32),
        pltpu.VMEM((D, F), F32),
        pltpu.VMEM((D, F), F32),
        pltpu.VMEM((F, D), F32),
        pltpu.VMEM((2 * DH, S), F32),
    ]
    outs = pl.pallas_call(
        kernel,
        grid=(S // TQ,),
        in_specs=in_specs,
        out_specs=out_specs,
        out_shape=out_shape,
        scratch_shapes=scratch,
        compiler_params=pltpu.CompilerParams(
            dimension_semantics=("arbitrary",),
            vmem_limit_bytes=110 * 1024 * 1024,
        ),
    )(*operands)
    h2, dx, dwq, dwk, dwv, dwo, dw1, dw3, dw2 = outs
    return (h2.reshape(1, S, D), dx.reshape(1, S, D), dwq, dwk, dwv, dwo, dw1, dw3, dw2)
```

```python
import jax
import jax.numpy as jnp
import jax.experimental.pallas as pl
import jax.experimental.pallas.tpu as pltpu

F32 = jnp.float32
BF16 = jnp.bfloat16

S = 2048
D = 512
H = 32
DH = 16
F = 1376
EPS = 1e-5
TQ = 256
TG = 2 * TQ
CH = 64
NCH = S // CH


def _dot(a, b):
    return jnp.dot(a, b, preferred_element_type=F32)


def _dot_nt(a, b):
    return jax.lax.dot_general(a, b, (((1,), (1,)), ((), ())), preferred_element_type=F32)


def _ln_stats_t(x):
    m = jnp.mean(x, axis=0, keepdims=True)
    xc = x - m
    var = jnp.mean(xc * xc, axis=0, keepdims=True)
    rstd = jax.lax.rsqrt(var + EPS)
    return xc * rstd, rstd


def _ln_bwd_t(dy, xhat, rstd):
    m1 = jnp.mean(dy, axis=0, keepdims=True)
    m2 = jnp.mean(dy * xhat, axis=0, keepdims=True)
    return rstd * (dy - m1 - xhat * m2)


def kernel(x_ref, g_ref,
           wq_ref, wqT_ref, wkv_ref, wkvT_ref, wo_ref, woT_ref,
           w1_ref, w1T_ref, w3_ref, w3T_ref, w2_ref, w2T_ref,
           h2_ref, dx_ref, dwq_ref, dwk_ref, dwv_ref, dwo_ref, dw1_ref, dw3_ref, dw2_ref,
           xT_s, aT_s, kT_s, vT_s, k_s, v_s,
           e_s, linv_s, q_s, o_s, do_s, dq_s, dxp_s,
           s_a, s_b, ds_a, ds_b,
           acc_wq, acc_wo, acc_w1, acc_w3, acc_w2, acc_kv):
    i = pl.program_id(0)
    nblk = pl.num_programs(0)

    @pl.when(i == 0)
    def _():
        for c in range(S // TQ):
            xt_b = x_ref[pl.ds(c * TQ, TQ), :].T
            xT_s[:, pl.ds(c * TQ, TQ)] = xt_b
            xhat, _ = _ln_stats_t(xt_b.astype(F32))
            aT_s[:, pl.ds(c * TQ, TQ)] = xhat.astype(BF16)
        kvT = _dot(wkvT_ref[...], aT_s[...]).astype(BF16)
        kT = kvT[0:DH, :]
        vT = kvT[DH:2 * DH, :]
        kT_s[...] = kT
        vT_s[...] = vT
        k_s[...] = kT.T
        v_s[...] = vT.T
        acc_wq[...] = jnp.zeros_like(acc_wq)
        acc_wo[...] = jnp.zeros_like(acc_wo)
        acc_w1[...] = jnp.zeros_like(acc_w1)
        acc_w3[...] = jnp.zeros_like(acc_w3)
        acc_w2[...] = jnp.zeros_like(acc_w2)
        acc_kv[...] = jnp.zeros_like(acc_kv)

    col0 = pl.multiple_of(i * TQ, TQ)
    aT = aT_s[:, pl.ds(col0, TQ)]
    xT = xT_s[:, pl.ds(col0, TQ)].astype(F32)

    q_s[...] = (_dot(wqT_ref[...], aT) * (DH ** -0.5)).astype(BF16)

    def scores_group(s_ref, j):
        h_a = 2 * j
        hsa = pl.multiple_of(h_a * DH, DH)
        hsb = pl.multiple_of((h_a + 1) * DH, DH)
        qg = jnp.concatenate([q_s[pl.ds(hsa, DH), :], q_s[pl.ds(hsb, DH), :]], axis=1)
        s_ref[...] = _dot(k_s[...], qg)

    def softmax_head(s_ref, off, h):
        hs = pl.multiple_of(h * DH, DH)
        m8 = jnp.max(s_ref[:, off:off + TQ].reshape(S // 8, 8, TQ), axis=0)
        m = jnp.max(m8, axis=0, keepdims=True)
        mb = jnp.broadcast_to(m, (8, TQ))
        l8 = jnp.zeros((8, TQ), F32)
        for c in range(NCH):
            cs = c * CH
            sc = s_ref[cs:cs + CH, off:off + TQ].reshape(CH // 8, 8, TQ)
            e = jnp.exp(sc - mb[None])
            l8 = l8 + jnp.sum(e, axis=0)
            e_s[h, cs:cs + CH, :] = e.reshape(CH, TQ).astype(BF16)
        linv = 1.0 / jnp.sum(l8, axis=0, keepdims=True)
        linv_s[h] = linv
        o_s[pl.ds(hs, DH), :] = _dot(vT_s[...], e_s[h]) * linv

    def fwd_quad(i, carry):
        ja = 2 * i
        jb = 2 * i + 1
        scores_group(s_b, jb)
        softmax_head(s_a, 0, 2 * ja)
        softmax_head(s_a, TQ, 2 * ja + 1)
        scores_group(s_a, ja + 2)
        softmax_head(s_b, 0, 2 * jb)
        softmax_head(s_b, TQ, 2 * jb + 1)
        return carry

    scores_group(s_a, jnp.int32(0))
    jax.lax.fori_loop(0, H // 4 - 1, fwd_quad, 0)
    scores_group(s_b, H // 2 - 1)
    softmax_head(s_a, 0, H - 4)
    softmax_head(s_a, TQ, H - 3)
    softmax_head(s_b, 0, H - 2)
    softmax_head(s_b, TQ, H - 1)

    o_f = o_s[...]
    o_b = o_f.astype(BF16)
    hT = xT + _dot(woT_ref[...], o_b)
    bT, rstd2 = _ln_stats_t(hT)
    b_b = bT.astype(BF16)
    gate = _dot(w1T_ref[...], b_b)
    up = _dot(w3T_ref[...], b_b)
    sig = jax.nn.sigmoid(gate)
    silu = gate * sig
    hh_b = (silu * up).astype(BF16)
    h2T = hT + _dot(w2T_ref[...], hh_b)
    h2_ref[...] = h2T.T.astype(BF16)

    gT = g_ref[...].T.astype(F32)
    g_b = gT.astype(BF16)
    dhh = _dot(w2_ref[...], g_b)
    acc_w2[...] += _dot_nt(hh_b, g_b)
    dgate = dhh * up * (sig * (1.0 + gate * (1.0 - sig)))
    dup = dhh * silu
    dgate_b = dgate.astype(BF16)
    dup_b = dup.astype(BF16)
    acc_w1[...] += _dot_nt(dgate_b, b_b)
    acc_w3[...] += _dot_nt(dup_b, b_b)
    dbT = _dot(w1_ref[...], dgate_b) + _dot(w3_ref[...], dup_b)
    dhT = gT + _ln_bwd_t(dbT, bT, rstd2)
    dh_b = dhT.astype(BF16)
    acc_wo[...] += _dot_nt(o_b, dh_b)
    do_s[...] = _dot(wo_ref[...], dh_b)

    def dp_group(s_ref, j):
        h_a = 2 * j
        hsa = pl.multiple_of(h_a * DH, DH)
        hsb = pl.multiple_of((h_a + 1) * DH, DH)
        dopa = (do_s[pl.ds(hsa, DH), :] * linv_s[h_a]).astype(BF16)
        dopb = (do_s[pl.ds(hsb, DH), :] * linv_s[h_a + 1]).astype(BF16)
        s_ref[...] = _dot(v_s[...], jnp.concatenate([dopa, dopb], axis=1))

    def ds_from(s_ref, off, ds_ref, h):
        hs = pl.multiple_of(h * DH, DH)
        dop = do_s[pl.ds(hs, DH), :] * linv_s[h]
        dpr = jnp.sum(dop * o_s[pl.ds(hs, DH), :], axis=0, keepdims=True)
        dprb = jnp.broadcast_to(dpr, (8, TQ))
        for c in range(NCH):
            cs = c * CH
            dpc = s_ref[cs:cs + CH, off:off + TQ].reshape(CH // 8, 8, TQ) - dprb[None]
            ec = e_s[h, cs:cs + CH, :].astype(F32).reshape(CH // 8, 8, TQ)
            ds_ref[cs:cs + CH, :] = (ec * dpc).reshape(CH, TQ).astype(BF16)

    def mm_head(ds_ref, h):
        hs = pl.multiple_of(h * DH, DH)
        dop_b = (do_s[pl.ds(hs, DH), :] * linv_s[h]).astype(BF16)
        dq_s[pl.ds(hs, DH), :] = _dot(kT_s[...], ds_ref[...]) * (DH ** -0.5)
        acc_kv[0:DH, :] += _dot_nt(q_s[pl.ds(hs, DH), :], ds_ref[...])
        acc_kv[DH:2 * DH, :] += _dot_nt(dop_b, e_s[h])

    def bwd_quad(i, carry):
        ja = 2 * i
        jb = 2 * i + 1
        dp_group(s_b, jb)
        ds_from(s_a, 0, ds_a, 2 * ja)
        mm_head(ds_a, 2 * ja)
        ds_from(s_a, TQ, ds_a, 2 * ja + 1)
        mm_head(ds_a, 2 * ja + 1)
        dp_group(s_a, ja + 2)
        ds_from(s_b, 0, ds_b, 2 * jb)
        mm_head(ds_b, 2 * jb)
        ds_from(s_b, TQ, ds_b, 2 * jb + 1)
        mm_head(ds_b, 2 * jb + 1)
        return carry

    dp_group(s_a, jnp.int32(0))
    jax.lax.fori_loop(0, H // 4 - 1, bwd_quad, 0)
    dp_group(s_b, H // 2 - 1)
    ds_from(s_a, 0, ds_a, H - 4)
    mm_head(ds_a, H - 4)
    ds_from(s_a, TQ, ds_b, H - 3)
    mm_head(ds_b, H - 3)
    ds_from(s_b, 0, ds_a, H - 2)
    mm_head(ds_a, H - 2)
    ds_from(s_b, TQ, ds_b, H - 1)
    mm_head(ds_b, H - 1)

    dq_b = dq_s[...].astype(BF16)
    acc_wq[...] += _dot_nt(aT, dq_b)
    daT = _dot(wq_ref[...], dq_b)
    xhat1, rstd1 = _ln_stats_t(xT)
    dxp_s[:, pl.ds(col0, TQ)] = dhT + _ln_bwd_t(daT, xhat1, rstd1)

    @pl.when(i == nblk - 1)
    def _():
        kv_b = acc_kv[...].astype(BF16)
        dwkvT = _dot_nt(kv_b, aT_s[...])
        dwk_ref[...] = dwkvT[0:DH, :].astype(BF16)
        dwv_ref[...] = dwkvT[DH:2 * DH, :].astype(BF16)
        for c in range(S // TQ):
            cs = c * TQ
            dakv = _dot(wkv_ref[...], kv_b[:, cs:cs + TQ])
            xhat_c, rstd_c = _ln_stats_t(xT_s[:, pl.ds(cs, TQ)].astype(F32))
            dxc = dxp_s[:, pl.ds(cs, TQ)] + _ln_bwd_t(dakv, xhat_c, rstd_c)
            dx_ref[pl.ds(cs, TQ), :] = dxc.T.astype(BF16)
        dwq_ref[...] = acc_wq[...].astype(BF16)
        dwo_ref[...] = acc_wo[...].astype(BF16)
        dw1_ref[...] = acc_w1[...].astype(BF16)
        dw3_ref[...] = acc_w3[...].astype(BF16)
        dw2_ref[...] = acc_w2[...].astype(BF16)


def _full(shape):
    return pl.BlockSpec(shape, lambda i: tuple(0 for _ in shape), pipeline_mode=pl.Buffered(1))


@jax.jit
def pallas_sequential_preLN__grouped_kv_mqa__glu_gated_swiglu__prompt_kernel(
        A_x, A_wq, A_wk, A_wv, A_wo, B_x, B_w1, B_w3, B_w2, grad_out):
    x = A_x.reshape(S, D)
    g = grad_out.reshape(S, D)
    wkv = jnp.concatenate([A_wk, A_wv], axis=1)
    operands = (x, g,
                A_wq, A_wq.T, wkv, wkv.T, A_wo, A_wo.T,
                B_w1, B_w1.T, B_w3, B_w3.T, B_w2, B_w2.T)
    in_specs = [
        _full((S, D)),
        pl.BlockSpec((TQ, D), lambda i: (i, 0)),
        _full((D, D)), _full((D, D)), _full((D, 2 * DH)), _full((2 * DH, D)),
        _full((D, D)), _full((D, D)),
        _full((D, F)), _full((F, D)), _full((D, F)), _full((F, D)), _full((F, D)), _full((D, F)),
    ]
    out_shape = (
        jax.ShapeDtypeStruct((S, D), BF16),
        jax.ShapeDtypeStruct((S, D), BF16),
        jax.ShapeDtypeStruct((D, D), BF16),
        jax.ShapeDtypeStruct((DH, D), BF16),
        jax.ShapeDtypeStruct((DH, D), BF16),
        jax.ShapeDtypeStruct((D, D), BF16),
        jax.ShapeDtypeStruct((F, D), BF16),
        jax.ShapeDtypeStruct((F, D), BF16),
        jax.ShapeDtypeStruct((F, D), BF16),
    )
    out_specs = (
        pl.BlockSpec((TQ, D), lambda i: (i, 0)),
        _full((S, D)), _full((D, D)), _full((DH, D)), _full((DH, D)), _full((D, D)),
        _full((F, D)), _full((F, D)), _full((F, D)),
    )
    scratch = [
        pltpu.VMEM((D, S), BF16),
        pltpu.VMEM((D, S), BF16),
        pltpu.VMEM((DH, S), BF16),
        pltpu.VMEM((DH, S), BF16),
        pltpu.VMEM((S, DH), BF16),
        pltpu.VMEM((S, DH), BF16),
        pltpu.VMEM((H, S, TQ), BF16),
        pltpu.VMEM((H, 1, TQ), F32),
        pltpu.VMEM((D, TQ), BF16),
        pltpu.VMEM((D, TQ), F32),
        pltpu.VMEM((D, TQ), F32),
        pltpu.VMEM((D, TQ), F32),
        pltpu.VMEM((D, S), F32),
        pltpu.VMEM((S, TG), F32),
        pltpu.VMEM((S, TG), F32),
        pltpu.VMEM((S, TQ), BF16),
        pltpu.VMEM((S, TQ), BF16),
        pltpu.VMEM((D, D), F32),
        pltpu.VMEM((D, D), F32),
        pltpu.VMEM((F, D), F32),
        pltpu.VMEM((F, D), F32),
        pltpu.VMEM((F, D), F32),
        pltpu.VMEM((2 * DH, S), F32),
    ]
    outs = pl.pallas_call(
        kernel,
        grid=(S // TQ,),
        in_specs=in_specs,
        out_specs=out_specs,
        out_shape=out_shape,
        scratch_shapes=scratch,
        compiler_params=pltpu.CompilerParams(
            dimension_semantics=("arbitrary",),
            vmem_limit_bytes=110 * 1024 * 1024,
        ),
    )(*operands)
    h2, dx, dwq, dwk, dwv, dwo, dw1, dw3, dw2 = outs
    return (h2.reshape(1, S, D), dx.reshape(1, S, D), dwq, dwk.T, dwv.T, dwo, dw1.T, dw3.T, dw2)
```
